```python
import os as _os
_os.environ.setdefault("JAX_PLATFORMS", "cpu")
import jax
import jax.numpy as jnp

def _softmax(x, axis=-1):
    return jax.nn.softmax(x, axis=axis)
def _gelu(x):
    return jax.nn.gelu(x, approximate=True)
def _silu(x):
    return jax.nn.silu(x)
def _sigmoid(x):
    return jax.nn.sigmoid(x)
def _layernorm(x, axis=-1, eps=1e-5):
    m = jnp.mean(x, axis=axis, keepdims=True)
    v = jnp.var(x, axis=axis, keepdims=True)
    return (x - m) / jnp.sqrt(v + eps)
def _scatter_add(tgt, idx, src, axis=0):
    return tgt.at[idx].add(src)
def _segment_sum(src, seg, n):
    return jax.ops.segment_sum(src, seg, n)
class _Rng:
    def __init__(self, key):
        self._k = key
    def _next(self):
        self._k, sub = jax.random.split(self._k)
        return sub
    def normal(self, shape):
        return jax.random.normal(self._next(), shape, dtype=jnp.bfloat16)
    def randint(self, lo, hi, shape):
        return jax.random.randint(self._next(), shape, lo, hi, dtype=jnp.int32)
    def uniform(self, shape, lo=0.0, hi=1.0):
        return jax.random.uniform(self._next(), shape, jnp.bfloat16, lo, hi)
    def permutation(self, n):
        return jax.random.permutation(self._next(), n)


kernel_name = 'concat_heads__sliding_block__grouped_kv_mqa__prompt'

def setup_inputs():
    _rng = _Rng(jax.random.key(int.from_bytes(__import__("os").urandom(4), "little")))
    _w = (lambda a: (lambda t: t.astype(jnp.bfloat16) if jnp.issubdtype(t.dtype, jnp.floating) else t)(jnp.asarray(a)))
    def _A_setup():
        B, S, D = 1, 2048, 576
        return {
            "x": _w((lambda *s: _rng.normal(s) * 0.2)(B, S, D)),
            "wqkv": _w((lambda *s: _rng.normal(s) * 0.2)(D, 3 * D)),
            "wo": _w((lambda *s: _rng.normal(s) * 0.05)(D, D)),
        }
    _A_in = _A_setup()

    def _B_setup():
        B, S, D, H = 1, 2048, 576, 32
        Dh = D // H
        return {
            "x": _w((lambda *s: _rng.normal(s) * 0.05)(B, S, D)),
            "wq": _w((lambda *s: _rng.normal(s) * 1.6)(D, H * Dh)),
            "wk": _w((lambda *s: _rng.normal(s) * 1.6)(D, Dh)),
            "wv": _w((lambda *s: _rng.normal(s) * 0.1)(D, Dh)),
            "wo": _w((lambda *s: _rng.normal(s) * 0.1)(H * Dh, D)),
        }
    _B_in = _B_setup()

    return {
        "A_x": _A_in["x"],
        "A_wqkv": _A_in["wqkv"],
        "A_wo": _A_in["wo"],
        "B_x": _B_in["x"],
        "B_wq": _B_in["wq"],
        "B_wk": _B_in["wk"],
        "B_wv": _B_in["wv"],
        "B_wo": _B_in["wo"],
    }

def reference(A_x, A_wqkv, A_wo, B_x, B_wq, B_wk, B_wv, B_wo):
    def _A_ref(x, wqkv, wo):
        B, S, D = x.shape
        H = 32; Dh = D // H; W = 256
        qkv = (lambda x, *d: x.transpose(*d))((x @ wqkv).reshape(B, S, 3, H, Dh), 2, 0, 3, 1, 4)
        q, k, v = qkv[0], qkv[1], qkv[2]
        scores = jnp.einsum("bhqd,bhkd->bhqk", q, k) * (Dh ** -0.5)
        idx = jnp.arange(S)
        mask = (idx[:, None] - idx[None, :] >= 0) & (idx[:, None] - idx[None, :] < W)
        scores = jnp.where(mask[None, None], scores, -1e9)
        p = _softmax(scores, axis=-1)
        o = jnp.einsum("bhqk,bhkd->bhqd", p, v)
        return (lambda x, *d: x.transpose(*d))(o, 0, 2, 1, 3).reshape(B, S, D) @ wo

    def _B_ref(x, wq, wk, wv, wo):
        B, S, D = x.shape
        H = 32
        Dh = D // H
        q = (lambda x, *d: x.transpose(*d))((x @ wq).reshape(B, S, H, Dh), 0, 2, 1, 3)
        k = x @ wk
        v = x @ wv
        scores = jnp.einsum("bhqd,bkd->bhqk", q, k) * (Dh ** -0.5)
        p = _softmax(scores, axis=-1)
        o = jnp.einsum("bhqk,bkd->bhqd", p, v)
        return (lambda x, *d: x.transpose(*d))(o, 0, 2, 1, 3).reshape(B, S, H * Dh) @ wo

    a = _A_ref(A_x, A_wqkv, A_wo)
    b = _B_ref(B_x, B_wq, B_wk, B_wv, B_wo)
    return jnp.concatenate([a, b], axis=-1)
```

```python
import functools
import math

import jax
import jax.numpy as jnp
import numpy as np
from jax.experimental import pallas as pl
from jax.experimental.pallas import tpu as pltpu

S = 2048
D = 576
H = 32
DH = 18
G = 4
NG = H // G
GR = G * DH
QB = 128
NQB = S // QB
W4 = G * QB
WIN = 256
NEG = -1e30
QSCALE = float(np.float32(0.2353515625) * np.float32(math.log2(math.e)))

NSUB = 4
STG = 0
FLUSH = 0
XCH = 512
BF = jnp.bfloat16
F32 = jnp.float32


def _kernel(ax_h, awqkv_h, awo_h, bx_h, bwq_h, bwk_h, bwv_h, bwo_h, out_h,
            ax, awqkv, awo, bx, bwq, bwk, bwv, bwo,
            wbt, wat, wot, wq, kb, vtb, ob, mb, ka, va, bias, stage, pa, zero,
            sem_in, sem_bx, sem_ax, sem_out, *bufs):
    sbufs = bufs[:2 * NSUB]
    sa = bufs[2 * NSUB:2 * NSUB + 2]
    ma = bufs[2 * NSUB + 2:2 * NSUB + 4]
    qw = bufs[2 * NSUB + 4:2 * NSUB + 6]
    oacc = bufs[2 * NSUB + 6:2 * NSUB + 8]
    ot = bufs[2 * NSUB + 8:2 * NSUB + 10]

    def cp(src, dst, sem):
        return pltpu.make_async_copy(src, dst, sem)

    d_bwq = cp(bwq_h, bwq, sem_in.at[0])
    d_bwk = cp(bwk_h, bwk, sem_in.at[1])
    d_bwv = cp(bwv_h, bwv, sem_in.at[2])
    d_awqkv = cp(awqkv_h, awqkv, sem_in.at[3])
    d_awo = cp(awo_h, awo, sem_in.at[4])
    d_bwo = cp(bwo_h, bwo, sem_in.at[5])

    def d_bx(c):
        return cp(bx_h.at[:, pl.ds(c * XCH, XCH)], bx.at[:, pl.ds(c * XCH, XCH)], sem_bx.at[c])

    def d_ax(c):
        return cp(ax_h.at[:, pl.ds(c * XCH, XCH)], ax.at[:, pl.ds(c * XCH, XCH)], sem_ax.at[c])

    d_bwq.start()
    d_bx(0).start()
    d_bwk.start()
    d_bwv.start()
    d_bx(1).start()

    zero[0] = 0
    for g in range(NG):
        ka[g, pl.ds(0, WIN), :] = jnp.zeros((WIN, 128), BF)
    for h in range(H):
        va[h, :, pl.ds(0, WIN)] = jnp.zeros((24, WIN), F32)
    rk = jax.lax.broadcasted_iota(jnp.int32, (QB, QB), 0)
    cq = jax.lax.broadcasted_iota(jnp.int32, (QB, QB), 1)
    bias[0] = jnp.where(rk <= cq, 0.0, NEG)
    bias[1] = jnp.where(rk > cq, 0.0, NEG)
    bias[2] = jnp.full((QB, QB), NEG, F32)

    d_bwq.wait()
    wbt[pl.ds(0, D), :] = bwq[...].T
    d_bwv.wait()
    wbt[pl.ds(D, 32), :] = jnp.concatenate([bwv[...], jnp.zeros((32 - DH, D), BF)], axis=0)
    d_bwk.wait()
    wbt[pl.ds(D + 32, 32), :] = jnp.concatenate([bwk[...], jnp.zeros((32 - DH, D), BF)], axis=0)

    def b_proj(c):
        d_bx(c).wait()
        if c == 0:
            d_bx(2).start()
            d_bx(3).start()
        elif c == 1:
            d_awqkv.start()
        elif c == 2:
            d_awo.start()
            d_bwo.start()
            d_ax(0).start()
        r0 = c * XCH
        res = jnp.dot(wbt[...], bx[:, pl.ds(r0, XCH)], preferred_element_type=F32)
        row32 = jax.lax.broadcasted_iota(jnp.int32, (32, QB), 0)
        for jj in range(XCH // QB):
            q = res[0:D + 16, jj * QB:(jj + 1) * QB] * QSCALE
            for g in range(NG):
                ws = []
                for i in range(G):
                    h = g * G + i
                    ws.append(jnp.where(row32 < DH, q[h * DH:h * DH + 32, :], 0.0))
                wq[(c * (XCH // QB) + jj) * NG + g] = jnp.concatenate(ws, axis=1).astype(BF)
        row24 = jax.lax.broadcasted_iota(jnp.int32, (24, XCH), 0)
        vtb[:, pl.ds(r0, XCH)] = jnp.where(row24 == DH, 1.0, res[D:D + 24, :])
        kt = jnp.concatenate([res[D + 32:D + 64, :], jnp.zeros((96, XCH), F32)], axis=0)
        kb[pl.ds(r0, XCH), :] = kt.T.astype(BF)

    for c in range(S // XCH):
        b_proj(c)

    NU = NQB * NG
    NSTEP = NU // NSUB

    def b_step(u_qk, s_w, u_pv, s_r, m, do_qk=True, do_pv=True):
        mn = acc = None
        if do_qk:
            w4 = jnp.concatenate([wq[u_qk], jnp.zeros((96, W4), BF)], axis=0)
        for c in range(S // 128):
            sl = slice(c * 128, (c + 1) * 128)
            if do_pv:
                p = jnp.exp2(s_r[sl, :] - m).astype(BF)
            if do_qk:
                s2 = jnp.dot(kb[sl, :], w4, preferred_element_type=F32)
                s_w[sl, :] = s2
                mc = jnp.max(s2.reshape(16, 8, W4), axis=0)
                mn = mc if mn is None else jnp.maximum(mn, mc)
            if do_pv:
                oo = jnp.dot(vtb[:, sl], p, preferred_element_type=F32)
                acc = oo if acc is None else acc + oo
        if do_pv:
            l = acc[DH:DH + 1, :]
            r = pl.reciprocal(l, approx=True)
            r = r * (2.0 - l * r)
            o = acc * r
            grp = jnp.concatenate([o[0:DH, i * QB:(i + 1) * QB] for i in range(G)], axis=0)
            ob[u_pv // NG, pl.ds(pl.multiple_of((u_pv % NG) * GR, 8), GR), :] = grp
        if do_qk:
            return jnp.max(mn, axis=0, keepdims=True)

    d_awqkv.wait()
    d_awo.wait()
    d_bwo.wait()
    d_ax(1).start()
    d_ax(2).start()
    d_ax(3).start()
    wat[...] = awqkv[...].T
    wot[pl.ds(0, D), :] = awo[...].T
    wot[pl.ds(D, D), :] = bwo[...].T
    for s in range(NSUB):
        mb[s:s + 1, :] = b_step(s, sbufs[s], None, None, None, do_pv=False)

    def b_body(i, carry):
        for par in range(2):
            @pl.when(i % 2 == par)
            def _():
                for s in range(NSUB):
                    r = sbufs[par * NSUB + s]
                    w = sbufs[(1 - par) * NSUB + s]
                    m = mb[par * NSUB + s:par * NSUB + s + 1, :]
                    u = i * NSUB + s
                    mm = b_step(u + NSUB, w, u, r, m)
                    mb[(1 - par) * NSUB + s:(1 - par) * NSUB + s + 1, :] = mm
        return carry

    jax.lax.fori_loop(0, NSTEP - 1, b_body, 0)

    d_ax(0).wait()

    def a_proj(j, par):
        r0 = j * QB if isinstance(j, int) else pl.multiple_of(j * QB, QB)
        res = jnp.dot(wat[...], ax[:, pl.ds(r0, QB)], preferred_element_type=F32)
        c0 = j * QB + WIN if isinstance(j, int) else pl.multiple_of(j * QB + WIN, QB)
        r80 = jax.lax.broadcasted_iota(jnp.int32, (80, QB), 0)
        for g in range(NG):
            qg = res[g * GR:g * GR + 80, :] * QSCALE
            ws = [jnp.where(jnp.logical_and(r80 >= i * DH, r80 < (i + 1) * DH), qg, 0.0) for i in range(G)]
            qw[par][g] = jnp.concatenate(ws, axis=1).astype(BF)
            ka[g, pl.ds(c0, QB), :] = res[D + g * GR:D + g * GR + 128, :].T.astype(BF)
        r24 = jax.lax.broadcasted_iota(jnp.int32, (24, QB), 0)
        for h in range(H):
            lo = 2 * D + h * DH
            if lo + 24 <= 3 * D:
                v = res[lo:lo + 24, :]
                v = jnp.where(r24 < DH, v, jnp.where(r24 == DH, 1.0, 0.0))
            else:
                v = res[3 * D - 24:3 * D, :]
                v = jnp.concatenate([v[24 - DH:24, :], jnp.ones((1, QB), F32), jnp.zeros((24 - DH - 1, QB), F32)], axis=0)
            va[h, :, pl.ds(c0, QB)] = v

    def a_stage(jq, jp, par_q, par_p):
        c0q = c0p = 3
        if jq is not None:
            rq = jq * QB if isinstance(jq, int) else pl.multiple_of(jq * QB, QB)
            c0q = max(0, 2 - jq) if isinstance(jq, int) else 0
        if jp is not None:
            rp = jp * QB if isinstance(jp, int) else pl.multiple_of(jp * QB, QB)
            c0p = max(0, 2 - jp) if isinstance(jp, int) else 0
            dz = zero[0]
        for g in range(NG):
            mn = None
            accs = [None] * G
            if jq is not None:
                w4 = jnp.concatenate([qw[par_q][g], jnp.zeros((48, W4), BF)], axis=0)
            if jp is not None:
                m = ma[par_p][g:g + 1, :]
            for c in range(3):
                sl = slice(c * QB, (c + 1) * QB)
                if c >= c0p:
                    p = jnp.exp2(sa[par_p][g, sl, :] - m).astype(BF)
                    if c == STG:
                        pa[dz + (g % 2)] = p
                        p = pa[(g % 2) + 2 * dz]
                if c >= c0q:
                    s2 = jnp.dot(ka[g, pl.ds(rq + c * QB, QB), :], w4, preferred_element_type=F32)
                    if c == 0:
                        b = bias[1] if isinstance(jq, int) else bias[jnp.where(jq >= 2, 1, 2)]
                        s2 = s2 + jnp.concatenate([b] * G, axis=1)
                    elif c == 2:
                        s2 = s2 + jnp.concatenate([bias[0]] * G, axis=1)
                    sa[par_q][g, sl, :] = s2
                    mc = jnp.max(s2.reshape(16, 8, W4), axis=0)
                    mn = mc if mn is None else jnp.maximum(mn, mc)
                if c >= c0p:
                    for i in range(G):
                        oo = jnp.dot(va[g * G + i, :, pl.ds(rp + c * QB, QB)], p[:, i * QB:(i + 1) * QB],
                                     preferred_element_type=F32)
                        accs[i] = oo if accs[i] is None else accs[i] + oo
            if jp is not None:
                oacc[par_p][g] = jnp.concatenate(accs, axis=1)
            if jq is not None:
                ma[par_q][g:g + 1, :] = jnp.max(mn, axis=0, keepdims=True)

    def normalize(acc):
        l = acc[DH:DH + 1, :]
        r = pl.reciprocal(l, approx=True)
        r = r * (2.0 - l * r)
        o = acc * r
        return jnp.concatenate([o[0:DH, i * QB:(i + 1) * QB] for i in range(G)], axis=0)

    def d_out(j, slot):
        r0 = j * QB if isinstance(j, int) else pl.multiple_of(j * QB, QB)
        return cp(stage.at[slot], out_h.at[pl.ds(r0, QB), :], sem_out.at[slot])

    def when(cond, fn):
        if isinstance(cond, bool):
            if cond:
                fn()
        else:
            pl.when(cond)(fn)

    def flush(j, slot):
        when(j >= 2, lambda: d_out(j - 2, slot).wait())
        stage[slot] = ot[slot][...].T
        d_out(j, slot).start()

    def out_proj(j, par):
        o_t = jnp.concatenate([normalize(oacc[par][g]) for g in range(NG)], axis=0).astype(BF)
        o_a = jnp.dot(wot[0:D, :], o_t, preferred_element_type=F32)
        o_b = jnp.dot(wot[D:2 * D, :], ob[j].astype(BF), preferred_element_type=F32)
        ot[par][pl.ds(0, D), :] = o_a.astype(BF)
        ot[par][pl.ds(D, D), :] = o_b.astype(BF)

    def a_block(t, par):
        def ok(j):
            return j if (not isinstance(t, int)) or 0 <= j < NQB else None
        if FLUSH == 0:
            if ok(t - 2) is not None:
                flush(t - 2, par)
            if ok(t + 1) is not None or ok(t) is not None:
                a_stage(ok(t + 1), ok(t), 1 - par, par)
            if ok(t + 2) is not None:
                a_proj(t + 2, par)
            if ok(t - 1) is not None:
                out_proj(t - 1, 1 - par)
        else:
            if ok(t + 1) is not None or ok(t) is not None:
                a_stage(ok(t + 1), ok(t), 1 - par, par)
            if ok(t - 1) is not None:
                out_proj(t - 1, 1 - par)
                flush(t - 1, 1 - par)
            if ok(t + 2) is not None:
                a_proj(t + 2, par)

    par = (NSTEP - 1) % 2
    ramp = [-2, -1]
    for s in range(NSUB):
        b_step(None, None, (NSTEP - 1) * NSUB + s, sbufs[par * NSUB + s],
               mb[par * NSUB + s:par * NSUB + s + 1, :], do_qk=False)
        if ramp and s % 2 == 0:
            tt = ramp.pop(0)
            a_block(tt, tt % 2)
    for tt in ramp:
        a_block(tt, tt % 2)

    a_block(0, 0)
    a_block(1, 1)

    def a_body(i, carry):
        for par in (0, 1):
            t = 2 * i + par

            @pl.when(jnp.logical_or(jnp.logical_or(t == 2, t == 6), t == 10))
            def _():
                d_ax((t + 2) // 4).wait()

            @pl.when(t >= 0)
            def _():
                a_block(t, par)
        return carry

    jax.lax.fori_loop(1, 7, a_body, 0)
    for t in range(14, NQB + 2 - FLUSH):
        a_block(t, t % 2)
    d_out(NQB - 2, 0).wait()
    d_out(NQB - 1, 1).wait()


def make_call():
    hbm = pl.BlockSpec(memory_space=pltpu.HBM)
    scratch = [
        pltpu.VMEM((D, S), BF), pltpu.VMEM((D, 3 * D), BF), pltpu.VMEM((D, D), BF),
        pltpu.VMEM((D, S), BF), pltpu.VMEM((D, D), BF), pltpu.VMEM((DH, D), BF),
        pltpu.VMEM((DH, D), BF), pltpu.VMEM((D, D), BF),
        pltpu.VMEM((D + 64, D), BF),
        pltpu.VMEM((3 * D, D), BF),
        pltpu.VMEM((2 * D, D), BF),
        pltpu.VMEM((NQB * NG, 32, W4), BF),
        pltpu.VMEM((S, 128), BF),
        pltpu.VMEM((24, S), F32),
        pltpu.VMEM((NQB, D, QB), F32),
        pltpu.VMEM((8, W4), F32),
        pltpu.VMEM((NG, S + WIN, 128), BF),
        pltpu.VMEM((H, 24, S + WIN), F32),
        pltpu.VMEM((3, QB, QB), F32),
        pltpu.VMEM((2, QB, 2 * D), BF),
        pltpu.VMEM((2, QB, W4), BF),
        pltpu.SMEM((1,), jnp.int32),
        pltpu.SemaphoreType.DMA((6,)),
        pltpu.SemaphoreType.DMA((4,)),
        pltpu.SemaphoreType.DMA((4,)),
        pltpu.SemaphoreType.DMA((2,)),
    ] + [pltpu.VMEM((S, W4), F32) for _ in range(2 * NSUB)] \
      + [pltpu.VMEM((NG, 3 * QB, W4), F32) for _ in range(2)] \
      + [pltpu.VMEM((NG, W4), F32) for _ in range(2)] \
      + [pltpu.VMEM((NG, 80, W4), BF) for _ in range(2)] \
      + [pltpu.VMEM((NG, 24, W4), F32) for _ in range(2)] \
      + [pltpu.VMEM((2 * D, QB), BF) for _ in range(2)]
    return pl.pallas_call(
        _kernel,
        out_shape=jax.ShapeDtypeStruct((S, 2 * D), BF),
        in_specs=[hbm] * 8,
        out_specs=hbm,
        scratch_shapes=scratch,
        compiler_params=pltpu.CompilerParams(vmem_limit_bytes=120 * 1024 * 1024),
        name="fused",
    )


@jax.jit
def pallas_concat_heads__sliding_block__grouped_kv_mqa__prompt_kernel(
        A_x, A_wqkv, A_wo, B_x, B_wq, B_wk, B_wv, B_wo):
    out = make_call()(A_x.reshape(S, D).T, A_wqkv, A_wo, B_x.reshape(S, D).T, B_wq, B_wk.T, B_wv.T, B_wo)
    return out.reshape(1, S, 2 * D)
```

```python
import functools
import math

import jax
import jax.numpy as jnp
import numpy as np
from jax.experimental import pallas as pl
from jax.experimental.pallas import tpu as pltpu

S = 2048
D = 576
H = 32
DH = 18
G = 4
NG = H // G
GR = G * DH
QB = 128
NQB = S // QB
W4 = G * QB
WIN = 256
NEG = -1e30
QSCALE = float(np.float32(0.2353515625) * np.float32(math.log2(math.e)))

NSUB = 4
STG = 0
AMERGE = 0
ASTRUCT = 0
DMAV = 0
TAILM = 0
TAILW = 1
BU = 8
SKIP = ""
UNROLL_A = 0
AHEAD = 0
DYN = 0
XCH = 512
BF = jnp.bfloat16
F32 = jnp.float32


def _kernel(ax_h, awqkv_h, awo_h, bx_h, bwq_h, bwk_h, bwv_h, bwo_h, out_h,
            ax, awqkv, awo, bx, bwq, bwk, bwv, bwo,
            wbt, wat, wot, wq, kb, vtb, ob, mb, ka, va, bias, stage, pa, zero,
            sem_in, sem_bx, sem_ax, sem_out, *bufs):
    sbufs = bufs[:2 * NSUB]
    sa = bufs[2 * NSUB:2 * NSUB + 2]
    ma = bufs[2 * NSUB + 2:2 * NSUB + 4]
    qw = bufs[2 * NSUB + 4:2 * NSUB + 6]
    oacc = bufs[2 * NSUB + 6:2 * NSUB + 8]
    ot = bufs[2 * NSUB + 8:2 * NSUB + 10]

    def cp(src, dst, sem):
        return pltpu.make_async_copy(src, dst, sem)

    d_bwq = cp(bwq_h, bwq, sem_in.at[0])
    d_bwk = cp(bwk_h, bwk, sem_in.at[1])
    d_bwv = cp(bwv_h, bwv, sem_in.at[2])
    d_awqkv = cp(awqkv_h, awqkv, sem_in.at[3])
    d_awo = cp(awo_h, awo, sem_in.at[4])
    d_bwo = cp(bwo_h, bwo, sem_in.at[5])

    def d_bx(c):
        return cp(bx_h.at[:, pl.ds(c * XCH, XCH)], bx.at[:, pl.ds(c * XCH, XCH)], sem_bx.at[c])

    def d_ax(c):
        return cp(ax_h.at[:, pl.ds(c * XCH, XCH)], ax.at[:, pl.ds(c * XCH, XCH)], sem_ax.at[c])

    d_bwq.start()
    d_bwk.start()
    d_bwv.start()

    zero[0] = 0
    for g in range(NG):
        ka[g, pl.ds(0, WIN), :] = jnp.zeros((WIN, 128), BF)
    for h in range(H):
        va[h, :, pl.ds(0, WIN)] = jnp.zeros((24, WIN), F32)
    rk = jax.lax.broadcasted_iota(jnp.int32, (QB, QB), 0)
    cq = jax.lax.broadcasted_iota(jnp.int32, (QB, QB), 1)
    bias[0] = jnp.where(rk <= cq, 0.0, NEG)
    bias[1] = jnp.where(rk > cq, 0.0, NEG)
    bias[2] = jnp.full((QB, QB), NEG, F32)

    d_bx(0).start()

    d_bwq.wait()
    d_bx(1).start()
    d_bx(2).start()
    d_bx(3).start()
    wbt[pl.ds(0, D), :] = bwq[...].T
    d_bwv.wait()
    wbt[pl.ds(D, 32), :] = jnp.concatenate([bwv[...], jnp.zeros((32 - DH, D), BF)], axis=0)
    d_bwk.wait()
    wbt[pl.ds(D + 32, 32), :] = jnp.concatenate([bwk[...], jnp.zeros((32 - DH, D), BF)], axis=0)

    def b_proj(c):
        if c == 0:
            d_bx(0).wait()
        elif c == 1:
            d_bx(1).wait()
            d_bx(2).wait()
            d_bx(3).wait()
            if DMAV == 0:
                d_awqkv.start()
                d_awo.start()
                d_bwo.start()
        r0 = c * XCH
        res = jnp.dot(wbt[...], bx[:, pl.ds(r0, XCH)], preferred_element_type=F32)
        row32 = jax.lax.broadcasted_iota(jnp.int32, (32, QB), 0)
        for jj in range(XCH // QB):
            q = res[0:D + 16, jj * QB:(jj + 1) * QB] * QSCALE
            for g in range(NG):
                ws = []
                for i in range(G):
                    h = g * G + i
                    ws.append(jnp.where(row32 < DH, q[h * DH:h * DH + 32, :], 0.0))
                wq[(c * (XCH // QB) + jj) * NG + g] = jnp.concatenate(ws, axis=1).astype(BF)
        row24 = jax.lax.broadcasted_iota(jnp.int32, (24, XCH), 0)
        vtb[:, pl.ds(r0, XCH)] = jnp.where(row24 == DH, 1.0, res[D:D + 24, :])
        kt = jnp.concatenate([res[D + 32:D + 64, :], jnp.zeros((96, XCH), F32)], axis=0)
        kb[pl.ds(r0, XCH), :] = kt.T.astype(BF)

    for c in range(S // XCH):
        b_proj(c)

    NU = NQB * NG
    NSTEP = NU // NSUB

    def normalize(acc):
        l = acc[DH:DH + 1, :]
        r = pl.reciprocal(l, approx=True)
        r = r * (2.0 - l * r)
        o = acc * r
        return jnp.concatenate([o[0:DH, i * QB:(i + 1) * QB] for i in range(G)], axis=0)

    def run(items):
        for f in items:
            f()

    def merge(*streams):
        tagged = []
        for si, st in enumerate(streams):
            for k, f in enumerate(st):
                tagged.append(((k + 0.5) / len(st), si, k, f))
        tagged.sort(key=lambda t: t[:3])
        return [t[3] for t in tagged]

    def b_items(u_qk, s_w, u_pv, s_r, m_in, m_out, do_qk=True, do_pv=True):
        st = {"mn": None, "acc": None}

        def chunk(c):
            sl = slice(c * 128, (c + 1) * 128)
            if c == 0:
                if do_qk:
                    st["w4"] = jnp.concatenate([wq[u_qk], jnp.zeros((96, W4), BF)], axis=0)
                if do_pv:
                    st["m"] = mb[m_in:m_in + 1, :]
            if do_pv:
                p = jnp.exp2(s_r[sl, :] - st["m"]).astype(BF)
            if do_qk:
                s2 = jnp.dot(kb[sl, :], st["w4"], preferred_element_type=F32)
                s_w[sl, :] = s2
                mc = jnp.max(s2.reshape(16, 8, W4), axis=0)
                st["mn"] = mc if st["mn"] is None else jnp.maximum(st["mn"], mc)
            if do_pv:
                oo = jnp.dot(vtb[:, sl], p, preferred_element_type=F32)
                st["acc"] = oo if st["acc"] is None else st["acc"] + oo
            if c == S // 128 - 1:
                if do_pv:
                    g8 = (u_pv % NG) * GR
                    g8 = g8 if isinstance(g8, int) else pl.multiple_of(g8, 8)
                    ob[u_pv // NG, pl.ds(g8, GR), :] = normalize(st["acc"])
                if do_qk:
                    mb[m_out:m_out + 1, :] = jnp.max(st["mn"], axis=0, keepdims=True)

        return [functools.partial(chunk, c) for c in range(S // 128)]

    def a_weights():
        d_awqkv.wait()
        d_awo.wait()
        d_bwo.wait()
        wat[...] = awqkv[...].T
        wot[pl.ds(0, D), :] = awo[...].T
        wot[pl.ds(D, D), :] = bwo[...].T

    if DMAV == 0:
        a_weights()
    else:
        d_awqkv.start()
        d_awo.start()
        d_bwo.start()
    for c in range(S // XCH):
        d_ax(c).start()
    NB = 2 * NSUB
    for s in range(NSUB):
        run(b_items(s, sbufs[s], None, None, None, s, do_pv=False))

    def b_sub(u, slot):
        w = (slot + NSUB) % NB
        run(b_items(u + NSUB, sbufs[w], u, sbufs[slot], slot, w))

    for s in range(NSUB):
        b_sub(s, s)

    if DMAV == 1:
        a_weights()
    n_loop = (NU - 2 * NSUB) // BU
    n_pre = NU - 2 * NSUB - n_loop * BU
    assert n_pre % NB == 0 and BU % NB == 0
    for s in range(n_pre):
        b_sub(NSUB + s, (NSUB + s) % NB)

    def b_body(i, carry):
        for s in range(BU):
            b_sub(NSUB + n_pre + i * BU + s, (NSUB + s) % NB)
        return carry

    jax.lax.fori_loop(0, n_loop, b_body, 0)

    for c in range(S // XCH):
        d_ax(c).wait()

    PR = 2 * GR

    def a_proj_items(j, par):
        r0 = j * QB if isinstance(j, int) else pl.multiple_of(j * QB, QB)
        c0 = j * QB + WIN if isinstance(j, int) else pl.multiple_of(j * QB + WIN, QB)

        def piece(k):
            res = jnp.dot(wat[pl.ds(k * PR, PR), :], ax[:, pl.ds(r0, QB)], preferred_element_type=F32)
            kind, g0 = k // 4, 2 * (k % 4)
            if kind == 0:
                r80 = jax.lax.broadcasted_iota(jnp.int32, (80, QB), 0)
                for gg in range(2):
                    qg = res[0:80, :] if gg == 0 else jnp.concatenate([res[GR:PR, :], jnp.zeros((8, QB), F32)], axis=0)
                    qg = qg * QSCALE
                    ws = [jnp.where(jnp.logical_and(r80 >= i * DH, r80 < (i + 1) * DH), qg, 0.0) for i in range(G)]
                    qw[par][g0 + gg] = jnp.concatenate(ws, axis=1).astype(BF)
            elif kind == 1:
                for gg in range(2):
                    kg = res[0:128, :] if gg == 0 else jnp.concatenate([res[GR:PR, :], jnp.zeros((56, QB), F32)], axis=0)
                    ka[g0 + gg, pl.ds(c0, QB), :] = kg.T.astype(BF)
            else:
                r24 = jax.lax.broadcasted_iota(jnp.int32, (24, QB), 0)
                for i in range(2 * G):
                    if i * DH + 24 <= PR:
                        v = res[i * DH:i * DH + 24, :]
                        v = jnp.where(r24 < DH, v, jnp.where(r24 == DH, 1.0, 0.0))
                    else:
                        v = jnp.concatenate([res[i * DH:(i + 1) * DH, :], jnp.ones((1, QB), F32),
                                             jnp.zeros((24 - DH - 1, QB), F32)], axis=0)
                    va[g0 * G + i, :, pl.ds(c0, QB)] = v

        return [functools.partial(piece, k) for k in range(3 * D // PR)]

    def a_stage_items(jq, jp, par_q, par_p):
        c0q = c0p = 3
        if jq is not None:
            rq = jq * QB if isinstance(jq, int) else pl.multiple_of(jq * QB, QB)
            c0q = max(0, 2 - jq) if isinstance(jq, int) else 0
        if jp is not None:
            rp = jp * QB if isinstance(jp, int) else pl.multiple_of(jp * QB, QB)
            c0p = max(0, 2 - jp) if isinstance(jp, int) else 0
        st = {}

        def dz():
            if "dz" not in st:
                st["dz"] = zero[0]
            return st["dz"] if DYN else 0

        def chunk(g, c):
            sl = slice(c * QB, (c + 1) * QB)
            if c == min(c0q, c0p):
                st["mn"] = None
                st["accs"] = [None] * G
                if jq is not None:
                    st["w4"] = jnp.concatenate([qw[par_q][g + dz()], jnp.zeros((48, W4), BF)], axis=0)
                if jp is not None:
                    st["m"] = ma[par_p][pl.ds(g + dz(), 1), :]
            if c >= c0p:
                def probs(gg, cc):
                    m = st["m"] if gg == g else ma[par_p][gg:gg + 1, :]
                    return jnp.exp2(sa[par_p][gg, pl.ds(cc * QB, QB), :] - m).astype(BF)

                if AHEAD and c0p == 0:
                    if c == 0:
                        if g == 0:
                            pa[zero[0]] = probs(0, 0)
                        p = pa[(g % 2) + 2 * zero[0]]
                    else:
                        p = probs(g, c)
                    if c == AHEAD and g + 1 < NG:
                        pa[zero[0] + ((g + 1) % 2)] = probs(g + 1, 0)
                else:
                    p = probs(g, c)
                    if c == STG:
                        pa[zero[0] + (g % 2)] = p
                        p = pa[(g % 2) + 2 * zero[0]]
            if c >= c0q:
                s2 = jnp.dot(ka[g, pl.ds(rq + c * QB, QB), :], st["w4"], preferred_element_type=F32)
                if c == 0:
                    b = bias[1] if isinstance(jq, int) else bias[jnp.where(jq >= 2, 1, 2)]
                    s2 = s2 + jnp.concatenate([b] * G, axis=1)
                elif c == 2:
                    s2 = s2 + jnp.concatenate([bias[0]] * G, axis=1)
                sa[par_q][g, sl, :] = s2
                mc = jnp.max(s2.reshape(16, 8, W4), axis=0)
                st["mn"] = mc if st["mn"] is None else jnp.maximum(st["mn"], mc)
            if c >= c0p:
                accs = st["accs"]
                for i in range(G):
                    oo = jnp.dot(va[g * G + i, :, pl.ds(rp + c * QB, QB)], p[:, i * QB:(i + 1) * QB],
                                 preferred_element_type=F32)
                    accs[i] = oo if accs[i] is None else accs[i] + oo
            if c == 2:
                if jp is not None:
                    oacc[par_p][g] = jnp.concatenate(st["accs"], axis=1)
                if jq is not None:
                    ma[par_q][g:g + 1, :] = jnp.max(st["mn"], axis=0, keepdims=True)

        def group(g):
            if jq is not None:
                w4 = jnp.concatenate([qw[par_q][g], jnp.zeros((48, W4), BF)], axis=0)
                nk = (3 - c0q) * QB
                s2 = jnp.dot(ka[g, pl.ds(rq + c0q * QB, nk), :], w4, preferred_element_type=F32)
                bs = [None, jnp.zeros((QB, QB), F32), bias[0]]
                if c0q == 0:
                    bs[0] = bias[1] if isinstance(jq, int) else bias[jnp.where(jq >= 2, 1, 2)]
                s2 = s2 + jnp.concatenate([jnp.concatenate(bs[c0q:], axis=0)] * G, axis=1)
                sa[par_q][g, pl.ds(c0q * QB, nk), :] = s2
                ma[par_q][g:g + 1, :] = jnp.max(jnp.max(s2.reshape(nk // 8, 8, W4), axis=0), axis=0, keepdims=True)
            if jp is not None:
                m = ma[par_p][g:g + 1, :]
                ps = []
                for c in range(c0p, 3):
                    p = jnp.exp2(sa[par_p][g, pl.ds(c * QB, QB), :] - m).astype(BF)
                    if c == 2 and c0p == 0:
                        pa[zero[0] + (g % 2)] = p
                        p = None
                    ps.append(p)
                if ps[-1] is None:
                    ps[-1] = pa[(g % 2) + 2 * zero[0]]
                p = jnp.concatenate(ps, axis=0)
                nk = (3 - c0p) * QB
                accs = [jnp.dot(va[g * G + i, :, pl.ds(rp + c0p * QB, nk)], p[:, i * QB:(i + 1) * QB],
                                preferred_element_type=F32) for i in range(G)]
                oacc[par_p][g] = jnp.concatenate(accs, axis=1)

        if ASTRUCT:
            return [functools.partial(group, g) for g in range(NG)]
        return [functools.partial(chunk, g, c) for g in range(NG) for c in range(min(c0q, c0p), 3)]

    def d_out(j):
        r0 = j * QB if isinstance(j, int) else pl.multiple_of(j * QB, QB)
        return cp(stage.at[j], out_h.at[pl.ds(r0, QB), :], sem_out.at[j])

    def when(cond, fn):
        if isinstance(cond, bool):
            if cond:
                fn()
        else:
            pl.when(cond)(fn)

    def flush(j, slot):
        stage[j] = ot[slot][...].T
        d_out(j).start()

    def out_items(j, par):
        def part_a():
            z = zero[0] if DYN else 0
            o_t = jnp.concatenate([normalize(oacc[par][g + z]) for g in range(NG)], axis=0).astype(BF)
            ot[par][pl.ds(0, D), :] = jnp.dot(wot[0:D, :], o_t, preferred_element_type=F32).astype(BF)

        def part_b():
            ot[par][pl.ds(D, D), :] = jnp.dot(wot[D:2 * D, :], ob[j].astype(BF), preferred_element_type=F32).astype(BF)

        return [part_a, part_b]

    def out_proj(j, par):
        run(out_items(j, par))

    def a_block(t, par):
        def ok(j):
            return j if (not isinstance(t, int)) or 0 <= j < NQB else None
        dyn = not isinstance(t, int)
        if ok(t - 2) is not None and not (dyn and "f" in SKIP):
            flush(t - 2, par)
        if (ok(t + 1) is not None or ok(t) is not None) and not (dyn and "a" in SKIP):
            run(a_stage_items(ok(t + 1), ok(t), 1 - par, par))
        if ok(t + 2) is not None and not (dyn and "p" in SKIP):
            run(a_proj_items(t + 2, par))
        if ok(t - 1) is not None and not (dyn and "o" in SKIP):
            out_proj(t - 1, 1 - par)

    def b_tail(s):
        u = NU - NSUB + s
        return b_items(None, None, u, sbufs[u % NB], u % NB, None, do_qk=False)

    tails = [b_tail(s) for s in range(NSUB)]
    run(merge(tails[0], a_proj_items(0, 0)))
    run(merge(tails[1], a_proj_items(1, 1)))
    run(merge(tails[2], a_stage_items(0, None, 0, None) + a_stage_items(1, None, 1, None)))
    run(merge(tails[3] + a_stage_items(None, 0, None, 0), a_proj_items(2, 0)))
    a_block(1, 1)

    def a_body(i, carry):
        for par in (0, 1):
            t = 2 * i + par
            if AMERGE:
                a_block(t, par)
            else:
                @pl.when(t >= 0)
                def _():
                    a_block(t, par)
        return carry

    if UNROLL_A:
        for t in range(2, 14):
            pl.when(zero[0] == 0)(functools.partial(a_block, t, t % 2))
    else:
        jax.lax.fori_loop(1, 7, a_body, 0)
    def tail():
        if TAILM:
            flush(13, 1)
            oa14, ob14 = out_items(14, 0)
            oa15, ob15 = out_items(15, 1)
            run(merge(a_stage_items(None, 15, None, 1), [ob14, oa14, ob15]))
            flush(14, 0)
            oa15()
            flush(15, 1)
        else:
            for t in range(15, NQB + 2):
                a_block(t, t % 2)

    if TAILW == 1:
        pl.when(zero[0] == 0)(lambda: a_block(14, 0))
        tail()
    elif TAILW == 2:
        a_block(14, 0)
        pl.when(zero[0] == 0)(tail)
    else:
        a_block(14, 0)
        tail()

    for j in range(NQB):
        if "f" in SKIP and 0 <= j <= 11:
            continue
        d_out(j).wait()


def make_call():
    hbm = pl.BlockSpec(memory_space=pltpu.HBM)
    scratch = [
        pltpu.VMEM((D, S), BF), pltpu.VMEM((D, 3 * D), BF), pltpu.VMEM((D, D), BF),
        pltpu.VMEM((D, S), BF), pltpu.VMEM((D, D), BF), pltpu.VMEM((DH, D), BF),
        pltpu.VMEM((DH, D), BF), pltpu.VMEM((D, D), BF),
        pltpu.VMEM((D + 64, D), BF),
        pltpu.VMEM((3 * D, D), BF),
        pltpu.VMEM((2 * D, D), BF),
        pltpu.VMEM((NQB * NG, 32, W4), BF),
        pltpu.VMEM((S, 128), BF),
        pltpu.VMEM((24, S), F32),
        pltpu.VMEM((NQB, D, QB), F32),
        pltpu.VMEM((8, W4), F32),
        pltpu.VMEM((NG, S + WIN, 128), BF),
        pltpu.VMEM((H, 24, S + WIN), F32),
        pltpu.VMEM((3, QB, QB), F32),
        pltpu.VMEM((NQB, QB, 2 * D), BF),
        pltpu.VMEM((2, QB, W4), BF),
        pltpu.SMEM((1,), jnp.int32),
        pltpu.SemaphoreType.DMA((6,)),
        pltpu.SemaphoreType.DMA((4,)),
        pltpu.SemaphoreType.DMA((4,)),
        pltpu.SemaphoreType.DMA((NQB,)),
    ] + [pltpu.VMEM((S, W4), F32) for _ in range(2 * NSUB)] \
      + [pltpu.VMEM((NG, 3 * QB, W4), F32) for _ in range(2)] \
      + [pltpu.VMEM((NG, W4), F32) for _ in range(2)] \
      + [pltpu.VMEM((NG, 80, W4), BF) for _ in range(2)] \
      + [pltpu.VMEM((NG, 24, W4), F32) for _ in range(2)] \
      + [pltpu.VMEM((2 * D, QB), BF) for _ in range(2)]
    return pl.pallas_call(
        _kernel,
        out_shape=jax.ShapeDtypeStruct((S, 2 * D), BF),
        in_specs=[hbm] * 8,
        out_specs=hbm,
        scratch_shapes=scratch,
        compiler_params=pltpu.CompilerParams(vmem_limit_bytes=120 * 1024 * 1024),
        name="fused",
    )


@jax.jit
def pallas_concat_heads__sliding_block__grouped_kv_mqa__prompt_kernel(
        A_x, A_wqkv, A_wo, B_x, B_wq, B_wk, B_wv, B_wo):
    out = make_call()(A_x.reshape(S, D).T, A_wqkv, A_wo, B_x.reshape(S, D).T, B_wq, B_wk.T, B_wv.T, B_wo)
    return out.reshape(1, S, 2 * D)
```
